```python
import os as _os
_os.environ.setdefault("JAX_PLATFORMS", "cpu")
import jax
import jax.numpy as jnp

def _softmax(x, axis=-1):
    return jax.nn.softmax(x, axis=axis)
def _gelu(x):
    return jax.nn.gelu(x, approximate=True)
def _silu(x):
    return jax.nn.silu(x)
def _sigmoid(x):
    return jax.nn.sigmoid(x)
def _layernorm(x, axis=-1, eps=1e-5):
    m = jnp.mean(x, axis=axis, keepdims=True)
    v = jnp.var(x, axis=axis, keepdims=True)
    return (x - m) / jnp.sqrt(v + eps)
def _scatter_add(tgt, idx, src, axis=0):
    return tgt.at[idx].add(src)
def _segment_sum(src, seg, n):
    return jax.ops.segment_sum(src, seg, n)
class _Rng:
    def __init__(self, key):
        self._k = key
    def _next(self):
        self._k, sub = jax.random.split(self._k)
        return sub
    def normal(self, shape):
        return jax.random.normal(self._next(), shape, dtype=jnp.bfloat16)
    def randint(self, lo, hi, shape):
        return jax.random.randint(self._next(), shape, lo, hi, dtype=jnp.int32)
    def uniform(self, shape, lo=0.0, hi=1.0):
        return jax.random.uniform(self._next(), shape, jnp.bfloat16, lo, hi)
    def permutation(self, n):
        return jax.random.permutation(self._next(), n)


kernel_name = 'gated_mix__mha_block__mha_block__prompt'

def setup_inputs():
    _rng = _Rng(jax.random.key(int.from_bytes(__import__("os").urandom(4), "little")))
    _w = (lambda a: (lambda t: t.astype(jnp.bfloat16) if jnp.issubdtype(t.dtype, jnp.floating) else t)(jnp.asarray(a)))
    def _A_setup():
        B, S, D, H = 1, 2048, 448, 16
        return {
            "x": _w((lambda *s: _rng.normal(s) * 0.05)(B, S, D)),
            "wqkv": _w((lambda *s: _rng.normal(s) * 0.4)(D, 3 * D)),
            "wo": _w((lambda *s: _rng.normal(s) * 0.05)(D, D)),
        }
    _A_in = _A_setup()

    def _B_setup():
        B, S, D, H = 1, 2048, 448, 16
        return {
            "x": _w((lambda *s: _rng.normal(s) * 0.05)(B, S, D)),
            "wqkv": _w((lambda *s: _rng.normal(s) * 0.4)(D, 3 * D)),
            "wo": _w((lambda *s: _rng.normal(s) * 0.05)(D, D)),
        }
    _B_in = _B_setup()

    return {
        "A_x": _A_in["x"],
        "A_wqkv": _A_in["wqkv"],
        "A_wo": _A_in["wo"],
        "B_x": _B_in["x"],
        "B_wqkv": _B_in["wqkv"],
        "B_wo": _B_in["wo"],
        "gate_w": _w((lambda *s: _rng.normal(s) * 0.05)(448) * 16.0),
    }

def reference(A_x, A_wqkv, A_wo, B_x, B_wqkv, B_wo, gate_w):
    def _A_ref(x, wqkv, wo):
        B, S, D = x.shape
        H = 16
        Dh = D // H
        qkv = (lambda x, *d: x.transpose(*d))((x @ wqkv).reshape(B, S, 3, H, Dh), 2, 0, 3, 1, 4)
        q, k, v = qkv[0], qkv[1], qkv[2]
        scores = jnp.einsum("bhqd,bhkd->bhqk", q, k) * (Dh ** -0.5)
        p = _softmax(scores, axis=-1)
        o = jnp.einsum("bhqk,bhkd->bhqd", p, v)
        return (lambda x, *d: x.transpose(*d))(o, 0, 2, 1, 3).reshape(B, S, D) @ wo

    def _B_ref(x, wqkv, wo):
        B, S, D = x.shape
        H = 16
        Dh = D // H
        qkv = (lambda x, *d: x.transpose(*d))((x @ wqkv).reshape(B, S, 3, H, Dh), 2, 0, 3, 1, 4)
        q, k, v = qkv[0], qkv[1], qkv[2]
        scores = jnp.einsum("bhqd,bhkd->bhqk", q, k) * (Dh ** -0.5)
        p = _softmax(scores, axis=-1)
        o = jnp.einsum("bhqk,bhkd->bhqd", p, v)
        return (lambda x, *d: x.transpose(*d))(o, 0, 2, 1, 3).reshape(B, S, D) @ wo

    x = A_x
    g = _sigmoid((x * gate_w).sum(-1, keepdims=True))
    a = _A_ref(x, A_wqkv, A_wo)
    b = _B_ref(x, B_wqkv, B_wo)
    return g * a + (1 - g) * b
```

```python
import functools, math
import jax
import jax.numpy as jnp
import jax.experimental.pallas as pl
import jax.experimental.pallas.tpu as pltpu

S, D, H, DH, DP = 2048, 448, 16, 28, 32
NH = 2 * H
NG = NH // 4
GW = 4 * DH
F32, BF16 = jnp.float32, jnp.bfloat16
NT = (((1,), (1,)), ((), ()))

def make_kernel(MQ=256, RA=512, RB=512, CK=256, LAG=2, UNR=16, OB=256, MERGE=1):
    QSCALE = (DH ** -0.5) * math.log2(math.e)
    NQB = S // MQ
    NU = NH * NQB
    NC = S // CK
    NRA = S // RA
    assert 0 < LAG < NC and UNR % 2 == 0

    def kernel(xt_hbm, wa_hbm, wb_hbm, woa_hbm, wob_hbm, gw_hbm, o_hbm,
               xt_ref, wa_ref, wb_ref, woa_ref, wob_ref, gw_ref, o_ref, sems, xsems, osems,
               wqv_scr, wk_scr, wo_scr, wot_scr, x_scr, qt_scr, k_scr, vt_scr, ot_scr, g_scr, sa_scr, sb_scr):
        cp_wa = pltpu.make_async_copy(wa_hbm, wa_ref, sems.at[0])
        cp_wb = pltpu.make_async_copy(wb_hbm, wb_ref, sems.at[1])
        cp_gw = pltpu.make_async_copy(gw_hbm, gw_ref, sems.at[2])
        cp_woa = pltpu.make_async_copy(woa_hbm, woa_ref, sems.at[3])
        cp_wob = pltpu.make_async_copy(wob_hbm, wob_ref, sems.at[4])
        cp_x = [pltpu.make_async_copy(xt_hbm.at[:, i * RA:(i + 1) * RA], xt_ref.at[:, i * RA:(i + 1) * RA], xsems.at[i])
                for i in range(NRA)]
        cp_wa.start()
        cp_gw.start()
        wqv_scr[0, 2 * D:, :] = jnp.zeros((16, D), BF16)
        wk_scr[...] = jnp.zeros(wk_scr.shape, BF16)
        wo_scr[...] = jnp.zeros(wo_scr.shape, BF16)
        qt_scr[:, :, GW:, :] = jnp.zeros((NQB, NG, 128 - GW, MQ), BF16)
        row = jax.lax.broadcasted_iota(jnp.int32, (NH, 16, S), 1)
        vt_scr[:, 16:, :] = jnp.where(row == DH - 16, 1.0, 0.0).astype(BF16)
        if not MERGE:
            sa_scr[...] = jnp.zeros(sa_scr.shape, F32)
            sb_scr[...] = jnp.zeros(sb_scr.shape, F32)

        def prep(b, w_ref):
            wt = w_ref[...].T
            wqv_scr[b, 0:D, :] = wt[0:D]
            wqv_scr[b, D:2 * D, :] = wt[2 * D:]
            for g in range(NG // 2):
                wk_scr[b, g * 128:g * 128 + GW, :] = wt[D + g * GW:D + (g + 1) * GW]

        def proj(b, i, RC):
            r0 = pl.multiple_of(i * RC, RC)
            rs = pl.ds(r0, RC)
            xtc = xt_ref[:, rs]
            if b == 0:
                xc = xtc.T
                x_scr[rs, :] = xc
            else:
                xc = x_scr[rs, :]
            kk = jax.lax.dot_general(xc, wk_scr[b], NT, preferred_element_type=F32)
            for g in range(NG // 2):
                k_scr[b * (NG // 2) + g, rs, :] = kk[:, g * 128:(g + 1) * 128].astype(BF16)
            nr = 2 * D + 16 if b == 0 else 2 * D
            qv = jnp.dot(wqv_scr[b, :nr, :], xtc, preferred_element_type=F32)
            qt = (qv[:D] * QSCALE).astype(BF16)
            for h in range(H):
                vt_scr[b * H + h, 0:DH, rs] = qv[D + h * DH:D + (h + 1) * DH].astype(BF16)
            if b == 0:
                gs = jax.nn.sigmoid(qv[2 * D:2 * D + 8])
            for t in range(RC // MQ):
                if b == 0:
                    g_scr[i * (RC // MQ) + t] = gs[:, t * MQ:(t + 1) * MQ]
                qt_scr[i * (RC // MQ) + t, b * (NG // 2):(b + 1) * (NG // 2), 0:GW, :] = (
                    qt[:, t * MQ:(t + 1) * MQ].reshape(NG // 2, GW, MQ))

        cp_wa.wait()
        for cp in cp_x:
            cp.start()
        cp_wb.start()
        cp_woa.start()
        cp_wob.start()
        prep(0, wa_ref)
        cp_gw.wait()
        wqv_scr[0, 2 * D:2 * D + 1, :] = gw_ref[...]
        def pa(i, c):
            r0 = pl.multiple_of(i * RA, RA)
            pltpu.make_async_copy(xt_hbm.at[:, pl.ds(r0, RA)], xt_ref.at[:, pl.ds(r0, RA)], xsems.at[i]).wait()
            proj(0, i, RA)
            return c
        jax.lax.fori_loop(0, NRA, pa, 0)

        def load_q(u):
            hh = u // NQB
            qb = u % NQB
            g = hh // 4
            j = hh % 4
            qg = qt_scr[qb, g]
            row = jax.lax.broadcasted_iota(jnp.int32, (128, MQ), 0)
            lo = j * DH
            return g, jnp.where((row >= lo) & (row < lo + DH), qg, jnp.zeros_like(qg))

        def qk_chunk(gq, c, s_ref, mpart):
            g, qm = gq
            kc = k_scr[g, c * CK:(c + 1) * CK, :]
            sT = jnp.dot(kc, qm, preferred_element_type=F32)
            s_ref[c * CK:(c + 1) * CK, :] = sT
            mc = jnp.max(sT.reshape(CK // 8, 8, MQ), axis=0)
            return mc if mpart is None else jnp.maximum(mpart, mc)

        def pv_chunk(u, c, s_ref, m, acc):
            hh = jnp.maximum(u, 0) // NQB
            p = jnp.exp2(s_ref[c * CK:(c + 1) * CK, :] - m).astype(BF16)
            d = jnp.dot(vt_scr[hh, :, c * CK:(c + 1) * CK], p, preferred_element_type=F32)
            return d if acc is None else acc + d

        def finish(u, acc):
            u = jnp.maximum(u, 0)
            hh = u // NQB
            qb = u % NQB
            gate = g_scr[qb][0:1, :]
            gate = jnp.where(hh < H, gate, 1.0 - gate)
            scale = gate / acc[DH:DH + 1, :]
            ot_scr[qb, hh] = (acc * scale).astype(BF16)

        def half(u1, s1_ref, s2_ref, m_prev2, acc_prev2, m_prev1, do_qk=True, do_p2=True, do_p1=True):
            if do_qk:
                gq = load_q(u1)
            mpart = None
            acc2 = acc_prev2
            acc1 = None
            for c in range(NC):
                if do_qk:
                    mpart = qk_chunk(gq, c, s1_ref, mpart)
                if c < LAG:
                    if do_p2:
                        acc2 = pv_chunk(u1 - 2, NC - LAG + c, s1_ref, m_prev2, acc2)
                        if c == LAG - 1:
                            finish(u1 - 2, acc2)
                elif do_p1:
                    acc1 = pv_chunk(u1 - 1, c - LAG, s2_ref, m_prev1, acc1)
            mnew = jnp.max(mpart, axis=0, keepdims=True) if do_qk else None
            return mnew, acc1

        bufs = (sa_scr, sb_scr)
        def steps(u0, n, carry):
            m2, acc2, m1_ = carry
            for t in range(n):
                s1, s2 = bufs[t % 2], bufs[(t + 1) % 2]
                mnew, acc1 = half(u0 + t, s1, s2, m2, acc2, m1_)
                m2, acc2, m1_ = m1_, acc1, mnew
            return m2, acc2, m1_

        cp_wb.wait()
        prep(1, wb_ref)
        cp_woa.wait()
        cp_wob.wait()
        for b, wo_ref in enumerate((woa_ref, wob_ref)):
            wo = wo_ref[...]
            for h in range(H):
                r = (b * H + h) * DP
                wo_scr[r:r + DH, :] = wo[h * DH:(h + 1) * DH]
        wot_scr[...] = wo_scr[...].T
        if MERGE:
            m0, _ = half(0, sa_scr, sb_scr, None, None, None, do_p2=False, do_p1=False)
            m1, acc0 = half(1, sb_scr, sa_scr, None, None, m0, do_p2=False)
        def pb(i, c):
            proj(1, i, RB)
            return c
        jax.lax.fori_loop(0, S // RB, pb, 0)

        if MERGE:
            nit = (NU - 2) // UNR
            rem = (NU - 2) - nit * UNR
            carry = jax.lax.fori_loop(0, nit, lambda it, c: steps(2 + it * UNR, UNR, c), (m0, acc0, m1))
            carry = steps(2 + nit * UNR, rem, carry)
        else:
            zm = jnp.zeros((1, MQ), F32)
            carry = jax.lax.fori_loop(0, NU // UNR, lambda it, c: steps(it * UNR, UNR, c),
                                      (zm, jnp.zeros((DP, MQ), F32), zm))
        m2, acc2, m1_ = carry
        _, acc1 = half(NU, sa_scr, sb_scr, m2, acc2, m1_, do_qk=False)
        half(NU + 1, sb_scr, sa_scr, m1_, acc1, None, do_qk=False, do_p1=False)

        def outp(i, c):
            cs = pl.ds(pl.multiple_of(i * OB, OB), OB)
            for t in range(OB // MQ):
                ot = ot_scr[i * (OB // MQ) + t].reshape(NH * DP, MQ)
                o = jnp.dot(wot_scr[...], ot, preferred_element_type=F32)
                o_ref[:, pl.ds(pl.multiple_of(i * OB + t * MQ, MQ), MQ)] = o.astype(o_ref.dtype)
            pltpu.make_async_copy(o_ref.at[:, cs], o_hbm.at[:, cs], osems.at[i]).start()
            return c
        jax.lax.fori_loop(0, S // OB, outp, 0)
        for i in range(S // OB):
            pltpu.make_async_copy(o_ref.at[:, i * OB:(i + 1) * OB], o_hbm.at[:, i * OB:(i + 1) * OB], osems.at[i]).wait()
    return kernel

_MQ = 256
_RA = 512
_RB = 1024
_CK = 256
_LAG = 2
_UNR = 16
_OB = 512
_MERGE = 1
_kernel = make_kernel(_MQ, _RA, _RB, _CK, _LAG, _UNR, _OB, _MERGE)
@jax.jit
def pallas_gated_mix__mha_block__mha_block__prompt_kernel(A_x, A_wqkv, A_wo, B_x, B_wqkv, B_wo, gate_w):
    xt = A_x.reshape(S, D).T
    out = pl.pallas_call(
        _kernel,
        out_shape=jax.ShapeDtypeStruct((D, S), BF16),
        in_specs=[pl.BlockSpec(memory_space=pl.ANY)] * 6,
        out_specs=pl.BlockSpec(memory_space=pl.ANY),
        scratch_shapes=[
            pltpu.VMEM((D, S), BF16),
            pltpu.VMEM((D, 3 * D), BF16),
            pltpu.VMEM((D, 3 * D), BF16),
            pltpu.VMEM((D, D), BF16),
            pltpu.VMEM((D, D), BF16),
            pltpu.VMEM((1, D), BF16),
            pltpu.VMEM((D, S), BF16),
            pltpu.SemaphoreType.DMA((5,)),
            pltpu.SemaphoreType.DMA((S // _RA,)),
            pltpu.SemaphoreType.DMA((S // _OB,)),
            pltpu.VMEM((2, 2 * D + 16, D), BF16),
            pltpu.VMEM((2, 512, D), BF16),
            pltpu.VMEM((1024, D), BF16),
            pltpu.VMEM((D, 1024), BF16),
            pltpu.VMEM((S, D), BF16),
            pltpu.VMEM((S // _MQ, NG, 128, _MQ), BF16),
            pltpu.VMEM((NG, S, 128), BF16),
            pltpu.VMEM((NH, DP, S), BF16),
            pltpu.VMEM((S // _MQ, NH, DP, _MQ), BF16),
            pltpu.VMEM((S // _MQ, 8, _MQ), F32),
            pltpu.VMEM((S, _MQ), F32),
            pltpu.VMEM((S, _MQ), F32),
        ],
        compiler_params=pltpu.CompilerParams(vmem_limit_bytes=100 * 1024 * 1024),
    )(xt, A_wqkv, B_wqkv, A_wo, B_wo, gate_w.reshape(1, D))
    return out.T.reshape(1, S, D)
```

```python
import math

import jax
import jax.numpy as jnp
import jax.experimental.pallas as pl
import jax.experimental.pallas.tpu as pltpu

S, D, H, DH = 2048, 448, 16, 28
DP = 32
NH = 2 * H
NG = NH // 4
GW = 4 * DH
F32, BF16 = jnp.float32, jnp.bfloat16
NT = (((1,), (1,)), ((), ()))

MQ = 256
CK = 128
LAG = 4
RA = 512
RB = 1024
OB = 512
NQB = S // MQ
NU = NH * NQB
NC = S // CK
NRA = S // RA
UNR = 2 * NQB
QSCALE = (DH ** -0.5) * math.log2(math.e)


def _kernel(xt_hbm, wa_hbm, wb_hbm, woa_hbm, wob_hbm, gw_hbm, o_hbm,
            xt_ref, wa_ref, wb_ref, woa_ref, wob_ref, gw_ref, o_ref, sems, xsems, osems,
            wqv_scr, wk_scr, wo_scr, wot_scr, x_scr, qt_scr, k_scr, vt_scr, ot_scr, g_scr,
            sa_scr, sb_scr, kbuf, vbuf):
    cp_wa = pltpu.make_async_copy(wa_hbm, wa_ref, sems.at[0])
    cp_wb = pltpu.make_async_copy(wb_hbm, wb_ref, sems.at[1])
    cp_gw = pltpu.make_async_copy(gw_hbm, gw_ref, sems.at[2])
    cp_woa = pltpu.make_async_copy(woa_hbm, woa_ref, sems.at[3])
    cp_wob = pltpu.make_async_copy(wob_hbm, wob_ref, sems.at[4])
    cp_x = [pltpu.make_async_copy(xt_hbm.at[:, i * RA:(i + 1) * RA],
                                  xt_ref.at[:, i * RA:(i + 1) * RA], xsems.at[i])
            for i in range(NRA)]
    cp_wa.start()
    cp_gw.start()
    cp_x[0].start()

    wqv_scr[0, 2 * D:, :] = jnp.zeros((16, D), BF16)
    wk_scr[...] = jnp.zeros(wk_scr.shape, BF16)
    wo_scr[...] = jnp.zeros(wo_scr.shape, BF16)
    qt_scr[:, :, GW:, :] = jnp.zeros((NQB, NG, 128 - GW, MQ), BF16)
    row = jax.lax.broadcasted_iota(jnp.int32, (NH, 16, S), 1)
    vt_scr[:, 16:, :] = jnp.where(row == DH - 16, 1.0, 0.0).astype(BF16)
    sa_scr[...] = jnp.zeros(sa_scr.shape, F32)
    sb_scr[...] = jnp.zeros(sb_scr.shape, F32)

    def prep(b, w_ref):
        wt = w_ref[...].T
        wqv_scr[b, 0:D, :] = wt[0:D]
        wqv_scr[b, D:2 * D, :] = wt[2 * D:]
        for g in range(NG // 2):
            wk_scr[b, g * 128:g * 128 + GW, :] = wt[D + g * GW:D + (g + 1) * GW]

    def proj(b, i, rc):
        rs = pl.ds(i * rc, rc)
        xtc = xt_ref[:, rs]
        if b == 0:
            xc = xtc.T
            x_scr[rs, :] = xc
        else:
            xc = x_scr[rs, :]
        kk = jax.lax.dot_general(xc, wk_scr[b], NT, preferred_element_type=F32)
        for g in range(NG // 2):
            k_scr[b * (NG // 2) + g, rs, :] = kk[:, g * 128:(g + 1) * 128].astype(BF16)
        nr = 2 * D + 16 if b == 0 else 2 * D
        qv = jnp.dot(wqv_scr[b, :nr, :], xtc, preferred_element_type=F32)
        qt = (qv[:D] * QSCALE).astype(BF16)
        for h in range(H):
            vt_scr[b * H + h, 0:DH, rs] = qv[D + h * DH:D + (h + 1) * DH].astype(BF16)
        if b == 0:
            gs = jax.nn.sigmoid(qv[2 * D:2 * D + 8])
        for t in range(rc // MQ):
            if b == 0:
                g_scr[i * (rc // MQ) + t] = gs[:, t * MQ:(t + 1) * MQ]
            qt_scr[i * (rc // MQ) + t, b * (NG // 2):(b + 1) * (NG // 2), 0:GW, :] = (
                qt[:, t * MQ:(t + 1) * MQ].reshape(NG // 2, GW, MQ))

    cp_wa.wait()
    for cp in cp_x[1:]:
        cp.start()
    cp_wb.start()
    cp_woa.start()
    cp_wob.start()
    prep(0, wa_ref)
    cp_gw.wait()
    wqv_scr[0, 2 * D:2 * D + 1, :] = gw_ref[...].reshape(1, D)
    for i in range(NRA):
        cp_x[i].wait()
        if i == NRA - 1:
            cp_wb.wait()
            prep(1, wb_ref)
        proj(0, i, RA)

    cp_woa.wait()
    cp_wob.wait()
    for b, wo_ref in enumerate((woa_ref, wob_ref)):
        wo = wo_ref[...]
        for h in range(H):
            r = (b * H + h) * DP
            wo_scr[r:r + DH, :] = wo[h * DH:(h + 1) * DH]
    wot_scr[...] = wo_scr[...].T
    for i in range(S // RB):
        proj(1, i, RB)

    def load_q(u):
        hh, qb, slot = u
        g = hh // 4
        lo = (hh % 4) * DH
        qg = qt_scr[qb, g]
        rows = jax.lax.broadcasted_iota(jnp.int32, (128, MQ), 0)
        qm = jnp.where((rows >= lo) & (rows < lo + DH), qg, jnp.zeros_like(qg))
        return (g if slot is None else None), qm

    def qk_chunk(gq, c, s_ref, mpart):
        g, qm = gq
        if g is None:
            kc = kbuf[c * CK:(c + 1) * CK, :]
        else:
            kc = k_scr[g, c * CK:(c + 1) * CK, :]
        st = jnp.dot(kc, qm, preferred_element_type=F32)
        s_ref[c * CK:(c + 1) * CK, :] = st
        mc = jnp.max(st.reshape(CK // 8, 8, MQ), axis=0)
        return mc if mpart is None else jnp.maximum(mpart, mc)

    def pv_chunk(u, c, s_ref, m, acc):
        hh, _, slot = u
        p = jnp.exp2(s_ref[c * CK:(c + 1) * CK, :] - m).astype(BF16)
        if slot is None:
            vt = vt_scr[hh, :, c * CK:(c + 1) * CK]
        else:
            vt = vbuf[slot, :, c * CK:(c + 1) * CK]
        d = jnp.dot(vt, p, preferred_element_type=F32)
        return d if acc is None else acc + d

    def finish(u, acc):
        hh, qb, _ = u
        gate = g_scr[qb][0:1, :]
        gate = jnp.where(hh < H, gate, 1.0 - gate)
        scale = gate / acc[DH:DH + 1, :]
        ot_scr[qb, hh] = (acc * scale).astype(BF16)

    def step(us, s1_ref, s2_ref, m_prev2, acc_prev2, m_prev1, do_qk=True, do_p1=True):
        u1, um1, um2 = us
        if do_qk:
            gq = load_q(u1)
        mpart = None
        acc2 = acc_prev2
        acc1 = None
        for c in range(NC):
            if do_qk:
                mpart = qk_chunk(gq, c, s1_ref, mpart)
            if c < LAG:
                acc2 = pv_chunk(um2, NC - LAG + c, s1_ref, m_prev2, acc2)
                if c == LAG - 1:
                    finish(um2, acc2)
            elif do_p1:
                acc1 = pv_chunk(um1, c - LAG, s2_ref, m_prev1, acc1)
        mnew = jnp.max(mpart, axis=0, keepdims=True) if do_qk else None
        return mnew, acc1

    def unit(hbase, off):
        dh = off // NQB
        hh = hbase + dh
        if isinstance(hbase, int):
            return hh, off % NQB, None
        if dh < 0:
            hh = jnp.maximum(hh, 0)
        return hh, off % NQB, dh + 1

    def units(hbase, off):
        return tuple(unit(hbase, off - k) for k in range(3))

    bufs = (sa_scr, sb_scr)

    def body(it, carry):
        hbase = it * 2
        m2, acc2, m1 = carry
        kbuf[...] = k_scr[hbase // 4]
        for k in range(3):
            vbuf[k] = vt_scr[jnp.maximum(hbase + k - 1, 0)]
        for t in range(UNR):
            mnew, acc1 = step(units(hbase, t), bufs[t % 2], bufs[(t + 1) % 2], m2, acc2, m1)
            m2, acc2, m1 = m1, acc1, mnew
        return m2, acc2, m1

    zm = jnp.zeros((1, MQ), F32)
    m2, acc2, m1 = jax.lax.fori_loop(0, NU // UNR, body, (zm, jnp.zeros((DP, MQ), F32), zm))
    _, acc1 = step(units(0, NU), sa_scr, sb_scr, m2, acc2, m1, do_qk=False)
    step(units(0, NU + 1), sb_scr, sa_scr, m1, acc1, None, do_qk=False, do_p1=False)

    def outp(i, c):
        cs = pl.ds(pl.multiple_of(i * OB, OB), OB)
        for t in range(OB // MQ):
            ot = ot_scr[i * (OB // MQ) + t].reshape(NH * DP, MQ)
            o = jnp.dot(wot_scr[...], ot, preferred_element_type=F32)
            o_ref[:, pl.ds(pl.multiple_of(i * OB + t * MQ, MQ), MQ)] = o.astype(o_ref.dtype)
        pltpu.make_async_copy(o_ref.at[:, cs], o_hbm.at[:, cs], osems.at[i]).start()
        return c
    jax.lax.fori_loop(0, S // OB, outp, 0)
    for i in range(S // OB):
        pltpu.make_async_copy(o_ref.at[:, i * OB:(i + 1) * OB],
                              o_hbm.at[:, i * OB:(i + 1) * OB], osems.at[i]).wait()


@jax.jit
def pallas_gated_mix__mha_block__mha_block__prompt_kernel(
    A_x: jax.Array,
    A_wqkv: jax.Array,
    A_wo: jax.Array,
    B_x: jax.Array,
    B_wqkv: jax.Array,
    B_wo: jax.Array,
    gate_w: jax.Array,
):
    del B_x
    xt = A_x.reshape(S, D).T
    out_t = pl.pallas_call(
        _kernel,
        out_shape=jax.ShapeDtypeStruct((D, S), BF16),
        in_specs=[pl.BlockSpec(memory_space=pl.ANY)] * 6,
        out_specs=pl.BlockSpec(memory_space=pl.ANY),
        scratch_shapes=[
            pltpu.VMEM((D, S), BF16),
            pltpu.VMEM((D, 3 * D), BF16),
            pltpu.VMEM((D, 3 * D), BF16),
            pltpu.VMEM((D, D), BF16),
            pltpu.VMEM((D, D), BF16),
            pltpu.VMEM((D,), BF16),
            pltpu.VMEM((D, S), BF16),
            pltpu.SemaphoreType.DMA((5,)),
            pltpu.SemaphoreType.DMA((NRA,)),
            pltpu.SemaphoreType.DMA((S // OB,)),
            pltpu.VMEM((2, 2 * D + 16, D), BF16),
            pltpu.VMEM((2, 512, D), BF16),
            pltpu.VMEM((NH * DP, D), BF16),
            pltpu.VMEM((D, NH * DP), BF16),
            pltpu.VMEM((S, D), BF16),
            pltpu.VMEM((NQB, NG, 128, MQ), BF16),
            pltpu.VMEM((NG, S, 128), BF16),
            pltpu.VMEM((NH, DP, S), BF16),
            pltpu.VMEM((NQB, NH, DP, MQ), BF16),
            pltpu.VMEM((NQB, 8, MQ), F32),
            pltpu.VMEM((S, MQ), F32),
            pltpu.VMEM((S, MQ), F32),
            pltpu.VMEM((S, 128), BF16),
            pltpu.VMEM((3, DP, S), BF16),
        ],
        compiler_params=pltpu.CompilerParams(vmem_limit_bytes=100 * 1024 * 1024),
    )(xt, A_wqkv, B_wqkv, A_wo, B_wo, gate_w)
    return out_t.T.reshape(1, S, D)
```

```python
import math

import jax
import jax.numpy as jnp
import jax.experimental.pallas as pl
import jax.experimental.pallas.tpu as pltpu

S, D, H, DH = 2048, 448, 16, 28
DP = 32
NH = 2 * H
NG = NH // 4
GW = 4 * DH
F32, BF16 = jnp.float32, jnp.bfloat16
NT = (((1,), (1,)), ((), ()))

MQ = 256
CK = 256
LAG = 2
RA = 512
RB = 512
OB = 256
NQB = S // MQ
NU = NH * NQB
NC = S // CK
NRA = S // RA
UNR = 4 * NQB
QSCALE = (DH ** -0.5) * math.log2(math.e)


def _kernel(xt_hbm, wa_hbm, wb_hbm, woa_hbm, wob_hbm, gw_hbm, o_hbm,
            xt_ref, wa_ref, wb_ref, woa_ref, wob_ref, gw_ref, o_ref, sems, xsems, osems,
            wt_scr, wo_scr, wot_scr, qt_scr, k_scr, vt_scr, ot_scr, g_scr,
            sa_scr, sb_scr, kbuf, vbuf):
    cp_wa = pltpu.make_async_copy(wa_hbm, wa_ref, sems.at[0])
    cp_wb = pltpu.make_async_copy(wb_hbm, wb_ref, sems.at[1])
    cp_gw = pltpu.make_async_copy(gw_hbm, gw_ref, sems.at[2])
    cp_woa = pltpu.make_async_copy(woa_hbm, woa_ref, sems.at[3])
    cp_wob = pltpu.make_async_copy(wob_hbm, wob_ref, sems.at[4])
    cp_x = [pltpu.make_async_copy(xt_hbm.at[:, i * RA:(i + 1) * RA],
                                  xt_ref.at[:, i * RA:(i + 1) * RA], xsems.at[i])
            for i in range(NRA)]
    cp_wa.start()
    cp_gw.start()
    cp_x[0].start()

    wt_scr[0, 3 * D:, :] = jnp.zeros((16, D), BF16)
    wo_scr[...] = jnp.zeros(wo_scr.shape, BF16)
    qt_scr[:, :, GW:, :] = jnp.zeros((NQB, NG, 128 - GW, MQ), BF16)
    row = jax.lax.broadcasted_iota(jnp.int32, (NH, 16, S), 1)
    vt_scr[:, 16:, :] = jnp.where(row == DH - 16, 1.0, 0.0).astype(BF16)
    sa_scr[...] = jnp.zeros(sa_scr.shape, F32)
    sb_scr[...] = jnp.zeros(sb_scr.shape, F32)

    def prep(b, w_ref):
        wt_scr[b, 0:3 * D, :] = w_ref[...].T

    def proj(b, i, rc):
        rs = pl.ds(i * rc, rc) if isinstance(i, int) else pl.ds(pl.multiple_of(i * rc, rc), rc)
        xtc = xt_ref[:, rs]
        nr = 3 * D + 16 if b == 0 else 3 * D
        qkv = jnp.dot(wt_scr[b, :nr, :], xtc, preferred_element_type=F32)
        qt = (qkv[:D] * QSCALE).astype(BF16)
        for g in range(NG // 2):
            kt = qkv[D + g * GW:D + g * GW + 128].astype(BF16)
            k_scr[b * (NG // 2) + g, rs, :] = kt.T
        for h in range(H):
            vt_scr[b * H + h, 0:DH, rs] = qkv[2 * D + h * DH:2 * D + (h + 1) * DH].astype(BF16)
        if b == 0:
            gs = jax.nn.sigmoid(qkv[3 * D:3 * D + 8])
        for t in range(rc // MQ):
            if b == 0:
                g_scr[i * (rc // MQ) + t] = gs[:, t * MQ:(t + 1) * MQ]
            qt_scr[i * (rc // MQ) + t, b * (NG // 2):(b + 1) * (NG // 2), 0:GW, :] = (
                qt[:, t * MQ:(t + 1) * MQ].reshape(NG // 2, GW, MQ))

    cp_wa.wait()
    for cp in cp_x[1:]:
        cp.start()
    cp_wb.start()
    cp_woa.start()
    cp_wob.start()
    prep(0, wa_ref)
    cp_gw.wait()
    wt_scr[0, 3 * D:3 * D + 1, :] = gw_ref[...].reshape(1, D)
    def pa(i, c):
        cs = pl.ds(pl.multiple_of(i * RA, RA), RA)
        pltpu.make_async_copy(xt_hbm.at[:, cs], xt_ref.at[:, cs], xsems.at[i]).wait()
        proj(0, i, RA)
        return c
    jax.lax.fori_loop(0, NRA - 1, pa, 0)
    cp_x[NRA - 1].wait()
    cp_wb.wait()
    prep(1, wb_ref)
    proj(0, NRA - 1, RA)

    def pb(i, c):
        proj(1, i, RB)
        return c
    jax.lax.fori_loop(0, S // RB, pb, 0)

    def load_q(u):
        hh, qb, slot = u
        g = hh // 4
        lo = (hh % 4) * DH
        qg = qt_scr[qb, g]
        rows = jax.lax.broadcasted_iota(jnp.int32, (128, MQ), 0)
        qm = jnp.where((rows >= lo) & (rows < lo + DH), qg, jnp.zeros_like(qg))
        return (g if slot is None else None), qm

    def qk_chunk(gq, c, s_ref, mpart):
        g, qm = gq
        if g is None:
            kc = kbuf[c * CK:(c + 1) * CK, :]
        else:
            kc = k_scr[g, c * CK:(c + 1) * CK, :]
        st = jnp.dot(kc, qm, preferred_element_type=F32)
        s_ref[c * CK:(c + 1) * CK, :] = st
        mc = jnp.max(st.reshape(CK // 8, 8, MQ), axis=0)
        return mc if mpart is None else jnp.maximum(mpart, mc)

    def pv_chunk(u, c, s_ref, m, acc):
        hh, _, slot = u
        p = jnp.exp2(s_ref[c * CK:(c + 1) * CK, :] - m).astype(BF16)
        if slot is None:
            vt = vt_scr[hh, :, c * CK:(c + 1) * CK]
        else:
            vt = vbuf[slot, :, c * CK:(c + 1) * CK]
        d = jnp.dot(vt, p, preferred_element_type=F32)
        return d if acc is None else acc + d

    def finish(u, acc):
        hh, qb, _ = u
        gate = g_scr[qb][0:1, :]
        gate = jnp.where(hh < H, gate, 1.0 - gate)
        scale = gate / acc[DH:DH + 1, :]
        ot_scr[qb, hh] = (acc * scale).astype(BF16)

    def step(us, s1_ref, s2_ref, m_prev2, acc_prev2, m_prev1, do_qk=True, do_p1=True):
        u1, um1, um2 = us
        if do_qk:
            gq = load_q(u1)
        mpart = None
        acc2 = acc_prev2
        acc1 = None
        for c in range(NC):
            if do_qk:
                mpart = qk_chunk(gq, c, s1_ref, mpart)
            if c < LAG:
                acc2 = pv_chunk(um2, NC - LAG + c, s1_ref, m_prev2, acc2)
                if c == LAG - 1:
                    finish(um2, acc2)
            elif do_p1:
                acc1 = pv_chunk(um1, c - LAG, s2_ref, m_prev1, acc1)
        mnew = jnp.max(mpart, axis=0, keepdims=True) if do_qk else None
        return mnew, acc1

    def unit(hbase, off):
        dh = off // NQB
        hh = hbase + dh
        if isinstance(hbase, int):
            return hh, off % NQB, None
        if dh < 0:
            hh = jnp.maximum(hh, 0)
        return hh, off % NQB, dh + 1

    def units(hbase, off):
        return tuple(unit(hbase, off - k) for k in range(3))

    bufs = (sa_scr, sb_scr)

    def body(it, carry):
        hbase = it * 4
        m2, acc2, m1 = carry
        kbuf[...] = k_scr[hbase // 4]
        for k in range(5):
            vbuf[k] = vt_scr[jnp.maximum(hbase + k - 1, 0)]
        for t in range(UNR):
            mnew, acc1 = step(units(hbase, t), bufs[t % 2], bufs[(t + 1) % 2], m2, acc2, m1)
            m2, acc2, m1 = m1, acc1, mnew
        return m2, acc2, m1

    zm = jnp.zeros((1, MQ), F32)
    m2, acc2, m1 = jax.lax.fori_loop(0, NU // UNR, body, (zm, jnp.zeros((DP, MQ), F32), zm))
    cp_woa.wait()
    cp_wob.wait()
    for b, wo_ref in enumerate((woa_ref, wob_ref)):
        wo = wo_ref[...]
        for h in range(H):
            r = (b * H + h) * DP
            wo_scr[r:r + DH, :] = wo[h * DH:(h + 1) * DH]
    wot_scr[...] = wo_scr[...].T
    _, acc1 = step(units(0, NU), sa_scr, sb_scr, m2, acc2, m1, do_qk=False)
    step(units(0, NU + 1), sb_scr, sa_scr, m1, acc1, None, do_qk=False, do_p1=False)

    def outp(i, c):
        cs = pl.ds(pl.multiple_of(i * OB, OB), OB)
        for t in range(OB // MQ):
            ot = ot_scr[i * (OB // MQ) + t].reshape(NH * DP, MQ)
            o = jnp.dot(wot_scr[...], ot, preferred_element_type=F32)
            o_ref[:, pl.ds(pl.multiple_of(i * OB + t * MQ, MQ), MQ)] = o.astype(o_ref.dtype)
        pltpu.make_async_copy(o_ref.at[:, cs], o_hbm.at[:, cs], osems.at[i]).start()
        return c
    jax.lax.fori_loop(0, S // OB, outp, 0)
    for i in range(S // OB):
        pltpu.make_async_copy(o_ref.at[:, i * OB:(i + 1) * OB],
                              o_hbm.at[:, i * OB:(i + 1) * OB], osems.at[i]).wait()


@jax.jit
def pallas_gated_mix__mha_block__mha_block__prompt_kernel(
    A_x: jax.Array,
    A_wqkv: jax.Array,
    A_wo: jax.Array,
    B_x: jax.Array,
    B_wqkv: jax.Array,
    B_wo: jax.Array,
    gate_w: jax.Array,
):
    del B_x
    xt = A_x.reshape(S, D).T
    out_t = pl.pallas_call(
        _kernel,
        out_shape=jax.ShapeDtypeStruct((D, S), BF16),
        in_specs=[pl.BlockSpec(memory_space=pl.ANY)] * 6,
        out_specs=pl.BlockSpec(memory_space=pl.ANY),
        scratch_shapes=[
            pltpu.VMEM((D, S), BF16),
            pltpu.VMEM((D, 3 * D), BF16),
            pltpu.VMEM((D, 3 * D), BF16),
            pltpu.VMEM((D, D), BF16),
            pltpu.VMEM((D, D), BF16),
            pltpu.VMEM((D,), BF16),
            pltpu.VMEM((D, S), BF16),
            pltpu.SemaphoreType.DMA((5,)),
            pltpu.SemaphoreType.DMA((NRA,)),
            pltpu.SemaphoreType.DMA((S // OB,)),
            pltpu.VMEM((2, 3 * D + 16, D), BF16),
            pltpu.VMEM((NH * DP, D), BF16),
            pltpu.VMEM((D, NH * DP), BF16),
            pltpu.VMEM((NQB, NG, 128, MQ), BF16),
            pltpu.VMEM((NG, S, 128), BF16),
            pltpu.VMEM((NH, DP, S), BF16),
            pltpu.VMEM((NQB, NH, DP, MQ), BF16),
            pltpu.VMEM((NQB, 8, MQ), F32),
            pltpu.VMEM((S, MQ), F32),
            pltpu.VMEM((S, MQ), F32),
            pltpu.VMEM((S, 128), BF16),
            pltpu.VMEM((5, DP, S), BF16),
        ],
        compiler_params=pltpu.CompilerParams(vmem_limit_bytes=100 * 1024 * 1024),
    )(xt, A_wqkv, B_wqkv, A_wo, B_wo, gate_w)
    return out_t.T.reshape(1, S, D)
```

```python
import math

import jax
import jax.numpy as jnp
import jax.experimental.pallas as pl
import jax.experimental.pallas.tpu as pltpu

S, D, H, DH = 2048, 448, 16, 28
DP = 32
NH = 2 * H
NG = NH // 4
GW = 4 * DH
F32, BF16 = jnp.float32, jnp.bfloat16

MQ = 256
CK = 256
LAG = 2
RA = 512
RB = 512
OB = 256
NQB = S // MQ
NU = NH * NQB
NC = S // CK
NRA = S // RA
UNR = 4 * NQB
QSCALE = (DH ** -0.5) * math.log2(math.e)


def _kernel(xt_hbm, wa_hbm, wb_hbm, woa_hbm, wob_hbm, gw_hbm, o_hbm,
            xt_ref, wa_ref, wb_ref, woa_ref, wob_ref, gw_ref, o_ref, sems, xsems, osems,
            wt_scr, wot_scr, qt_scr, k_scr, vt_scr, ot_scr, g_scr,
            sa_scr, sb_scr, kbuf, vbuf):
    cp_wa = pltpu.make_async_copy(wa_hbm, wa_ref, sems.at[0])
    cp_wb = pltpu.make_async_copy(wb_hbm, wb_ref, sems.at[1])
    cp_gw = pltpu.make_async_copy(gw_hbm, gw_ref, sems.at[2])
    cp_woa = pltpu.make_async_copy(woa_hbm, woa_ref, sems.at[3])
    cp_wob = pltpu.make_async_copy(wob_hbm, wob_ref, sems.at[4])
    cp_x = [pltpu.make_async_copy(xt_hbm.at[:, i * RA:(i + 1) * RA],
                                  xt_ref.at[:, i * RA:(i + 1) * RA], xsems.at[i])
            for i in range(NRA)]
    cp_wa.start()
    cp_gw.start()
    cp_x[0].start()

    wt_scr[0, 3 * D:, :] = jnp.zeros((16, D), BF16)
    qt_scr[:, :, GW:, :] = jnp.zeros((NQB, NG, 128 - GW, MQ), BF16)
    row = jax.lax.broadcasted_iota(jnp.int32, (NH, 16, S), 1)
    vt_scr[:, 16:, :] = jnp.where(row == DH - 16, 1.0, 0.0).astype(BF16)
    sa_scr[...] = jnp.zeros(sa_scr.shape, F32)
    sb_scr[...] = jnp.zeros(sb_scr.shape, F32)

    def prep(b, w_ref):
        wt_scr[b, 0:3 * D, :] = w_ref[...].T

    def proj(b, i, rc):
        rs = pl.ds(i * rc, rc) if isinstance(i, int) else pl.ds(pl.multiple_of(i * rc, rc), rc)
        xtc = xt_ref[:, rs]
        nr = 3 * D + 16 if b == 0 else 3 * D
        qkv = jnp.dot(wt_scr[b, :nr, :], xtc, preferred_element_type=F32)
        qt = (qkv[:D] * QSCALE).astype(BF16)
        for g in range(NG // 2):
            kt = qkv[D + g * GW:D + g * GW + 128].astype(BF16)
            k_scr[b * (NG // 2) + g, rs, :] = kt.T
        for h in range(H):
            vt_scr[b * H + h, 0:DH, rs] = qkv[2 * D + h * DH:2 * D + (h + 1) * DH].astype(BF16)
        if b == 0:
            gs = jax.nn.sigmoid(qkv[3 * D:3 * D + 8])
        for t in range(rc // MQ):
            if b == 0:
                g_scr[i * (rc // MQ) + t] = gs[:, t * MQ:(t + 1) * MQ]
            qt_scr[i * (rc // MQ) + t, b * (NG // 2):(b + 1) * (NG // 2), 0:GW, :] = (
                qt[:, t * MQ:(t + 1) * MQ].reshape(NG // 2, GW, MQ))

    cp_wa.wait()
    for cp in cp_x[1:]:
        cp.start()
    cp_wb.start()
    cp_woa.start()
    cp_wob.start()
    prep(0, wa_ref)
    cp_gw.wait()
    wt_scr[0, 3 * D:3 * D + 1, :] = gw_ref[...].reshape(1, D)
    def pa(i, c):
        cs = pl.ds(pl.multiple_of(i * RA, RA), RA)
        pltpu.make_async_copy(xt_hbm.at[:, cs], xt_ref.at[:, cs], xsems.at[i]).wait()
        proj(0, i, RA)
        return c
    jax.lax.fori_loop(0, NRA - 1, pa, 0)
    cp_x[NRA - 1].wait()
    cp_wb.wait()
    prep(1, wb_ref)
    proj(0, NRA - 1, RA)

    def pb(i, c):
        proj(1, i, RB)
        return c
    jax.lax.fori_loop(0, S // RB, pb, 0)

    def load_q(u):
        hh, qb, slot = u
        g = hh // 4
        lo = (hh % 4) * DH
        qg = qt_scr[qb, g]
        rows = jax.lax.broadcasted_iota(jnp.int32, (128, MQ), 0)
        qm = jnp.where((rows >= lo) & (rows < lo + DH), qg, jnp.zeros_like(qg))
        return (g if slot is None else None), qm

    def qk_chunk(gq, c, s_ref, mpart):
        g, qm = gq
        if g is None:
            kc = kbuf[c * CK:(c + 1) * CK, :]
        else:
            kc = k_scr[g, c * CK:(c + 1) * CK, :]
        st = jnp.dot(kc, qm, preferred_element_type=F32)
        s_ref[c * CK:(c + 1) * CK, :] = st
        mc = jnp.max(st.reshape(CK // 8, 8, MQ), axis=0)
        return mc if mpart is None else jnp.maximum(mpart, mc)

    def pv_chunk(u, c, s_ref, m, acc):
        hh, _, slot = u
        p = jnp.exp2(s_ref[c * CK:(c + 1) * CK, :] - m).astype(BF16)
        if slot is None:
            vt = vt_scr[hh, :, c * CK:(c + 1) * CK]
        else:
            vt = vbuf[slot, :, c * CK:(c + 1) * CK]
        d = jnp.dot(vt, p, preferred_element_type=F32)
        return d if acc is None else acc + d

    def finish(u, acc):
        hh, qb, slot = u
        j = hh % 4 if slot is None else (slot - 1) % 4
        gate = g_scr[qb][0:1, :]
        gate = jnp.where(hh < H, gate, 1.0 - gate)
        scale = gate / acc[DH:DH + 1, :]
        ot_scr[qb, hh // 4, j * DH:(j + 1) * DH, :] = (acc[:DH] * scale).astype(BF16)

    def step(us, s1_ref, s2_ref, m_prev2, acc_prev2, m_prev1, do_qk=True, do_p1=True):
        u1, um1, um2 = us
        if do_qk:
            gq = load_q(u1)
        mpart = None
        acc2 = acc_prev2
        acc1 = None
        for c in range(NC):
            if do_qk:
                mpart = qk_chunk(gq, c, s1_ref, mpart)
            if c < LAG:
                acc2 = pv_chunk(um2, NC - LAG + c, s1_ref, m_prev2, acc2)
                if c == LAG - 1:
                    finish(um2, acc2)
            elif do_p1:
                acc1 = pv_chunk(um1, c - LAG, s2_ref, m_prev1, acc1)
        mnew = jnp.max(mpart, axis=0, keepdims=True) if do_qk else None
        return mnew, acc1

    def unit(hbase, off):
        dh = off // NQB
        hh = hbase + dh
        if isinstance(hbase, int):
            return hh, off % NQB, None
        if dh < 0:
            hh = jnp.maximum(hh, 0)
        return hh, off % NQB, dh + 1

    def units(hbase, off):
        return tuple(unit(hbase, off - k) for k in range(3))

    bufs = (sa_scr, sb_scr)

    def body(it, carry):
        hbase = it * 4
        m2, acc2, m1 = carry
        kbuf[...] = k_scr[hbase // 4]
        for k in range(5):
            vbuf[k] = vt_scr[jnp.maximum(hbase + k - 1, 0)]
        for t in range(UNR):
            mnew, acc1 = step(units(hbase, t), bufs[t % 2], bufs[(t + 1) % 2], m2, acc2, m1)
            m2, acc2, m1 = m1, acc1, mnew
        return m2, acc2, m1

    zm = jnp.zeros((1, MQ), F32)
    m2, acc2, m1 = jax.lax.fori_loop(0, NU // UNR, body, (zm, jnp.zeros((DP, MQ), F32), zm))
    cp_woa.wait()
    cp_wob.wait()
    wot_scr[...] = jnp.concatenate([woa_ref[...], wob_ref[...]], axis=0).T
    _, acc1 = step(units(0, NU), sa_scr, sb_scr, m2, acc2, m1, do_qk=False)
    step(units(0, NU + 1), sb_scr, sa_scr, m1, acc1, None, do_qk=False, do_p1=False)

    def outp(i, c):
        cs = pl.ds(pl.multiple_of(i * OB, OB), OB)
        for t in range(OB // MQ):
            ot = ot_scr[i * (OB // MQ) + t].reshape(2 * D, MQ)
            o = jnp.dot(wot_scr[...], ot, preferred_element_type=F32)
            o_ref[:, pl.ds(pl.multiple_of(i * OB + t * MQ, MQ), MQ)] = o.astype(o_ref.dtype)
        pltpu.make_async_copy(o_ref.at[:, cs], o_hbm.at[:, cs], osems.at[i]).start()
        return c
    jax.lax.fori_loop(0, S // OB, outp, 0)
    for i in range(S // OB):
        pltpu.make_async_copy(o_ref.at[:, i * OB:(i + 1) * OB],
                              o_hbm.at[:, i * OB:(i + 1) * OB], osems.at[i]).wait()


@jax.jit
def pallas_gated_mix__mha_block__mha_block__prompt_kernel(
    A_x: jax.Array,
    A_wqkv: jax.Array,
    A_wo: jax.Array,
    B_x: jax.Array,
    B_wqkv: jax.Array,
    B_wo: jax.Array,
    gate_w: jax.Array,
):
    del B_x
    xt = A_x.reshape(S, D).T
    out_t = pl.pallas_call(
        _kernel,
        out_shape=jax.ShapeDtypeStruct((D, S), BF16),
        in_specs=[pl.BlockSpec(memory_space=pl.ANY)] * 6,
        out_specs=pl.BlockSpec(memory_space=pl.ANY),
        scratch_shapes=[
            pltpu.VMEM((D, S), BF16),
            pltpu.VMEM((D, 3 * D), BF16),
            pltpu.VMEM((D, 3 * D), BF16),
            pltpu.VMEM((D, D), BF16),
            pltpu.VMEM((D, D), BF16),
            pltpu.VMEM((D,), BF16),
            pltpu.VMEM((D, S), BF16),
            pltpu.SemaphoreType.DMA((5,)),
            pltpu.SemaphoreType.DMA((NRA,)),
            pltpu.SemaphoreType.DMA((S // OB,)),
            pltpu.VMEM((2, 3 * D + 16, D), BF16),
            pltpu.VMEM((D, 2 * D), BF16),
            pltpu.VMEM((NQB, NG, 128, MQ), BF16),
            pltpu.VMEM((NG, S, 128), BF16),
            pltpu.VMEM((NH, DP, S), BF16),
            pltpu.VMEM((NQB, NG, GW, MQ), BF16),
            pltpu.VMEM((NQB, 8, MQ), F32),
            pltpu.VMEM((S, MQ), F32),
            pltpu.VMEM((S, MQ), F32),
            pltpu.VMEM((S, 128), BF16),
            pltpu.VMEM((5, DP, S), BF16),
        ],
        compiler_params=pltpu.CompilerParams(vmem_limit_bytes=100 * 1024 * 1024),
    )(xt, A_wqkv, B_wqkv, A_wo, B_wo, gate_w)
    return out_t.T.reshape(1, S, D)
```
